```python
import os as _os
_os.environ.setdefault("JAX_PLATFORMS", "cpu")
import jax
import jax.numpy as jnp

def _softmax(x, axis=-1):
    return jax.nn.softmax(x, axis=axis)
def _gelu(x):
    return jax.nn.gelu(x, approximate=True)
def _silu(x):
    return jax.nn.silu(x)
def _sigmoid(x):
    return jax.nn.sigmoid(x)
def _layernorm(x, axis=-1, eps=1e-5):
    m = jnp.mean(x, axis=axis, keepdims=True)
    v = jnp.var(x, axis=axis, keepdims=True)
    return (x - m) / jnp.sqrt(v + eps)
def _scatter_add(tgt, idx, src, axis=0):
    return tgt.at[idx].add(src)
def _segment_sum(src, seg, n):
    return jax.ops.segment_sum(src, seg, n)
class _Rng:
    def __init__(self, key):
        self._k = key
    def _next(self):
        self._k, sub = jax.random.split(self._k)
        return sub
    def normal(self, shape):
        return jax.random.normal(self._next(), shape, dtype=jnp.bfloat16)
    def randint(self, lo, hi, shape):
        return jax.random.randint(self._next(), shape, lo, hi, dtype=jnp.int32)
    def uniform(self, shape, lo=0.0, hi=1.0):
        return jax.random.uniform(self._next(), shape, jnp.bfloat16, lo, hi)
    def permutation(self, n):
        return jax.random.permutation(self._next(), n)


kernel_name = 'parallel_sum__ssm_conv_s4__mixer_channel_mlp__prompt'

def setup_inputs():
    _rng = _Rng(jax.random.key(int.from_bytes(__import__("os").urandom(4), "little")))
    _w = (lambda a: (lambda t: t.astype(jnp.bfloat16) if jnp.issubdtype(t.dtype, jnp.floating) else t)(jnp.asarray(a)))
    def _A_setup():
        B, L, D, N = 1, 2048, 512, 128
        A_re = -jnp.exp((lambda *s: _rng.normal(s) * 0.1)(D, N))
        A_im = jnp.pi * (lambda *s: _rng.normal(s) * 0.1)(D, N)
        B_re = (lambda *s: _rng.normal(s) * 0.1)(D, N)
        B_im = (lambda *s: _rng.normal(s) * 0.1)(D, N)
        C_re = (lambda *s: _rng.normal(s) * 0.1)(D, N)
        C_im = (lambda *s: _rng.normal(s) * 0.1)(D, N)
        log_dt = (lambda *s: _rng.normal(s) * 0.1)(D) * 0.5 - 4.0
        Dskip = (lambda *s: _rng.normal(s) * 0.05)(D)
        return {
            "u": _w((lambda *s: _rng.normal(s) * 0.05)(B, L, D)),
            "A_re": _w(A_re),
            "A_im": _w(A_im),
            "B_re": _w(B_re),
            "B_im": _w(B_im),
            "C_re": _w(C_re),
            "C_im": _w(C_im),
            "log_dt": _w(log_dt),
            "Dskip": _w(Dskip),
        }
    _A_in = _A_setup()

    def _B_setup():
        B, S, D, F = 1, 2048, 512, 1792
        return {
            "x": _w((lambda *s: _rng.normal(s) * 0.05)(B, S, D)),
            "w1": _w((lambda *s: _rng.normal(s) * 0.2)(D, F) * (D ** -0.5)),
            "b1": _w((lambda *s: _rng.normal(s) * 0.2)(F)),
            "w2": _w((lambda *s: _rng.normal(s) * 0.2)(F, D) * (F ** -0.5)),
            "b2": _w((lambda *s: _rng.normal(s) * 0.05)(D)),
        }
    _B_in = _B_setup()

    return {
        "A_u": _A_in["u"],
        "A_A_re": _A_in["A_re"],
        "A_A_im": _A_in["A_im"],
        "A_B_re": _A_in["B_re"],
        "A_B_im": _A_in["B_im"],
        "A_C_re": _A_in["C_re"],
        "A_C_im": _A_in["C_im"],
        "A_log_dt": _A_in["log_dt"],
        "A_Dskip": _A_in["Dskip"],
        "B_x": _B_in["x"],
        "B_w1": _B_in["w1"],
        "B_b1": _B_in["b1"],
        "B_w2": _B_in["w2"],
        "B_b2": _B_in["b2"],
    }

def reference(A_u, A_A_re, A_A_im, A_B_re, A_B_im, A_C_re, A_C_im, A_log_dt, A_Dskip, B_x, B_w1, B_b1, B_w2, B_b2):
    def _A_ref(u, A_re, A_im, B_re, B_im, C_re, C_im, log_dt, Dskip):
        Bsz, L, D = u.shape
        dt = jnp.exp(log_dt)[:, None]
        A = A_re + 1j * A_im
        Bc = B_re + 1j * B_im
        Cc = C_re + 1j * C_im
        logdA = dt * A
        dB = dt * Bc
        l = (lambda x, dt: x.astype(dt))(jnp.arange(L), A_re.dtype)
        P = jnp.exp(logdA[:, :, None] * l[None, None, :])
        K = jnp.einsum("dn,dnl,dn->dl", Cc, P, dB).real
        L2 = 2 * L
        Kp = jnp.pad(K, ((0, 0), (0, L)))
        up = (lambda x, *d: x.transpose(*d))(u, 0, 2, 1)
        up = jnp.pad(up, ((0, 0), (0, 0), (0, L)))
        Kf = (lambda x, axes=(-2,-1): jnp.fft.rfft2(x.astype(jnp.float32), axes=axes))(Kp[:, None, :], axes=(-2, -1))
        Uf = (lambda x, axes=(-2,-1): jnp.fft.rfft2(x.astype(jnp.float32), axes=axes))(up[:, :, None, :], axes=(-2, -1))
        Yf = Uf * Kf[None, :, :, :]
        y = (lambda x, s, axes=(-2,-1): jnp.fft.irfft2(x, s=s, axes=axes).astype(jnp.bfloat16))(Yf, (1, L2), axes=(-2, -1))[:, :, 0, :L]
        y = (lambda x, *d: x.transpose(*d))(y, 0, 2, 1) + u * Dskip[None, None, :]
        return y

    def _B_ref(x, w1, b1, w2, b2):
        y = _layernorm(x, axis=-1)
        h = _gelu(jnp.einsum("bsd,df->bsf", y, w1) + b1)
        return jnp.einsum("bsf,fd->bsd", h, w2) + b2

    x = A_u
    xn = _layernorm(x, axis=-1)
    return x + _A_ref(xn, A_A_re, A_A_im, A_B_re, A_B_im, A_C_re, A_C_im, A_log_dt, A_Dskip) + _B_ref(xn, B_w1, B_b1, B_w2, B_b2)
```

```python
import functools
import jax
import jax.numpy as jnp
from jax import lax
import jax.experimental.pallas as pl
import jax.experimental.pallas.tpu as pltpu

f32, bf16, u32, i32 = jnp.float32, jnp.bfloat16, jnp.uint32, jnp.int32

L, D, N, F = 2048, 512, 128, 1792
Q, NC = 64, 32
TS = 513
US = 17
SS = 33
MB = 256
NB = L // MB
FC = 256
NF = F // FC
NP = 256


def cmul(ar, ai, br, bi):
    return ar * br - ai * bi, ar * bi + ai * br


def csq(ar, ai):
    return ar * ar - ai * ai, (ar * ai) * 2.0


def sincos(x):
    k = jnp.round(x * 0.6366197723675814)
    r = ((x - k * 1.5703125) - k * 4.837512969970703125e-4) - k * 7.54978995489188e-8
    z = r * r
    s = r + r * z * (-1.6666654611e-1 + z * (8.3321608736e-3 + z * -1.9515295891e-4))
    c = 1.0 + z * (-0.5 + z * (4.166664568298827e-2 + z * (-1.388731625493765e-3 + z * 2.443315711809948e-5)))
    q = k.astype(i32)
    swap = (q & 1) == 1
    sn = jnp.where(swap, c, s)
    cs = jnp.where(swap, s, c)
    sn = jnp.where((q & 2) == 2, -sn, sn)
    cs = jnp.where(((q + 1) & 2) == 2, -cs, cs)
    return sn, cs


def interleave(*gens):
    gens = [(g, n) for g, n in gens if n > 0]
    done = [0] * len(gens)
    total = sum(n for _, n in gens)
    for _ in range(total):
        best = min((i for i in range(len(gens)) if done[i] < gens[i][1]),
                   key=lambda i: (done[i] + 0.5) / gens[i][1])
        next(gens[best][0])
        done[best] += 1
    for g, n in gens:
        for _ in g:
            raise RuntimeError("generator not exhausted")


def chain(*gens):
    def it():
        for g, n in gens:
            for _ in range(n):
                next(g)
                yield
            for _ in g:
                raise RuntimeError("generator not exhausted")
    return it(), sum(n for _, n in gens)


def kernel(x_hbm, are_hbm, aim_hbm, bre_hbm, bim_hbm, cre_hbm, cim_hbm, ldt_hbm, dsk_hbm,
           w1_hbm, b1_hbm, w2_hbm, b2_hbm, o_hbm,
           xs, prm, v_ldt, v_dsk, v_b2, b1s, w1s, w2s, w1p, w2p, xnb, U, tab, l8, mu, SL, S2, Y, msk, ACC, ob,
           sem_x, sem_w1, sem_w2, sem_p, sem_v, sem_o, *, cfg):
    G2 = cfg.get("G2", (1, 4, 6))

    def cp_x(b):
        return pltpu.make_async_copy(x_hbm.at[pl.ds(b * MB, MB)], xs.at[pl.ds(b * MB, MB)], sem_x.at[b])

    def cp_w1(f):
        return pltpu.make_async_copy(w1_hbm.at[:, pl.ds(f * FC, FC)], w1s.at[:, pl.ds(f * FC, FC)], sem_w1.at[f])

    def cp_w2(f):
        return pltpu.make_async_copy(w2_hbm.at[pl.ds(f * FC, FC)], w2s.at[pl.ds(f * FC, FC)], sem_w2.at[f])

    p_hbm = [are_hbm, aim_hbm, bre_hbm, bim_hbm, cre_hbm, cim_hbm]

    def cp_p(i):
        return pltpu.make_async_copy(p_hbm[i], prm.at[i], sem_p.at[i])

    vec = [v_ldt, v_dsk, v_b2, b1s]
    v_hbm = [ldt_hbm, dsk_hbm, b2_hbm, b1_hbm]

    def cp_v(i):
        return pltpu.make_async_copy(v_hbm[i], vec[i], sem_v.at[i])

    def cp_o(b):
        return pltpu.make_async_copy(ob.at[pl.ds(b * MB, MB)], o_hbm.at[pl.ds(b * MB, MB)], sem_o.at[b])

    cp_x(0).start()
    cp_w1(0).start()
    for i in range(4):
        cp_v(i).start()
    cp_w2(0).start()
    for f in range(1, NF):
        cp_w1(f).start()
        cp_w2(f).start()
        if f == cfg.get("x1_after", 3):
            cp_x(1).start()
    for b in range(2, NB):
        cp_x(b).start()
    for i in range(6):
        cp_p(i).start()

    z = jnp.uint32(0)
    kk = lax.broadcasted_iota(i32, (32, 128), 0) * 2
    ln = lax.broadcasted_iota(i32, (32, 128), 1)
    lo = jnp.uint32(0x0000FFFF)
    hi = jnp.uint32(0xFFFF0000)
    for h in range(2):
        inh = (ln >= 64 * h) & (ln < 64 * h + 64)
        li = ln - 64 * h
        msk[h] = jnp.where(inh & (li >= kk), lo, z) | jnp.where(inh & (li >= kk + 1), hi, z)
    lane = lax.broadcasted_iota(i32, (16, 128), 1)
    laneA = jnp.where(lane < 64, jnp.uint32(0xFFFFFFFF), z)
    lane32 = lax.broadcasted_iota(i32, (32, 128), 1)
    row8 = lax.broadcasted_iota(i32, (8, 128), 0)
    c1 = 0.7978845608028654
    c12 = 0.7978845608028654 * 0.044715

    for i in range(4):
        cp_v(i).wait()
    dsk = v_dsk[...].astype(f32).reshape(1, D)
    b2 = v_b2[...].astype(f32).reshape(1, D)
    b1 = b1s[...].astype(f32).reshape(1, F)

    def ln_rows(k):
        r0 = k * 128
        x = xs[pl.ds(r0, 128), :].astype(f32)
        m = jnp.mean(x, axis=-1, keepdims=True)
        xc = x - m
        v = jnp.mean(xc * xc, axis=-1, keepdims=True)
        xn = xc * lax.rsqrt(v + 1e-5)
        xnb[pl.ds(r0 // 2, 64), :] = pltpu.bitcast(xn.astype(bf16), u32)
        pk = pltpu.pack_elementwise([xn[0:64], xn[64:128]], packed_dtype=bf16)
        for g in range(2):
            t = jnp.concatenate([pk[:, 128 * g:128 * g + 128], pk[:, 128 * (g + 2):128 * (g + 2) + 128]], axis=0)
            U[pl.ds(g * 128 * US + k, 128, stride=US), :] = t.T

    def g_ln(blocks):
        for b in blocks:
            cp_x(b).wait()
            for k in (2 * b, 2 * b + 1):
                ln_rows(k)
                yield

    def param_rows(dtc, r0, R):
        sl = pl.ds(r0, R)
        dtb = dtc[r0:r0 + R]
        ar = dtb * prm[0, sl, :].astype(f32)
        ai = dtb * prm[1, sl, :].astype(f32)
        dbr = dtb * prm[2, sl, :].astype(f32)
        dbi = dtb * prm[3, sl, :].astype(f32)
        wr, wi = cmul(prm[4, sl, :].astype(f32), prm[5, sl, :].astype(f32), dbr, dbi)
        wi = -wi
        e = jnp.exp(ar)
        sn, cs = sincos(ai)
        l1r, l1i = e * cs, e * sn
        l2r, l2i = csq(l1r, l1i)
        l4r, l4i = csq(l2r, l2i)
        l8r, l8i = csq(l4r, l4i)
        l3r, l3i = cmul(l2r, l2i, l1r, l1i)
        l5r, l5i = cmul(l4r, l4i, l1r, l1i)
        l6r, l6i = cmul(l4r, l4i, l2r, l2i)
        l7r, l7i = cmul(l4r, l4i, l3r, l3i)
        pw = [(jnp.ones_like(ar), jnp.zeros_like(ar)), (l1r, l1i), (l2r, l2i), (l3r, l3i),
              (l4r, l4i), (l5r, l5i), (l6r, l6i), (l7r, l7i), (l8r, l8i)]
        for s in range(8):
            tab[pl.ds((2 * 8 + s) * TS + r0, R), :] = pw[s][0]
            tab[pl.ds((3 * 8 + s) * TS + r0, R), :] = pw[s][1]
            pr, pi = pw[8 - s]
            tab[pl.ds((0 * 8 + s) * TS + r0, R), :] = wr * pr + wi * pi
            tab[pl.ds((1 * 8 + s) * TS + r0, R), :] = wi * pr - wr * pi
        l8[0, sl, :] = l8r
        l8[1, sl, :] = l8i
        mr, mi = csq(l8r, l8i)
        mr, mi = csq(mr, mi)
        mr, mi = csq(mr, mi)
        mu[0, sl, :] = mr
        mu[1, sl, :] = -mi
        mu[2, sl, :] = wr
        mu[3, sl, :] = wi

    PR = 16

    def g_param():
        for i in range(6):
            cp_p(i).wait()
        dt_row = jnp.exp(v_ldt[...].astype(f32).reshape(1, D)).astype(bf16).astype(f32)
        dtc = jnp.broadcast_to(dt_row, (128, D)).T
        for r0 in range(0, D, PR):
            param_rows(dtc, r0, PR)
            yield

    def bc(ref, part, d):
        return jnp.broadcast_to(ref[part, pl.ds(d, 1), :], (8, 128))

    def vgen(p, conj):
        t0 = 0 if conj else 2
        r_l, i_l = [], []
        for h in range(2):
            d = p + 256 * h
            tr = tab[pl.ds(t0 * 8 * TS + d, 8, stride=TS), :]
            ti = tab[pl.ds((t0 + 1) * 8 * TS + d, 8, stride=TS), :]
            sr, si = bc(l8, 0, d), bc(l8, 1, d)
            rs, is_ = [tr], [ti]
            for v in range(7):
                if conj:
                    tr, ti = tr * sr + ti * si, ti * sr - tr * si
                else:
                    tr, ti = tr * sr - ti * si, tr * si + ti * sr
                rs.append(tr)
                is_.append(ti)
            if conj:
                rs, is_ = rs[::-1], is_[::-1]
            r_l += rs
            i_l += is_
        return jnp.concatenate([jnp.concatenate(r_l, axis=0), jnp.concatenate(i_l, axis=0)], axis=1).astype(bf16)

    def p1_pair(p):
        Wb = vgen(p, True)
        u = U[pl.ds(p * US, 16), :]
        ua = u & laneA
        ub = u ^ ua
        lhs = pltpu.bitcast(jnp.concatenate([ua, ub], axis=0), bf16)
        s = jnp.dot(lhs, Wb, preferred_element_type=f32)
        for h in range(2):
            d = p + 256 * h
            for part in range(2):
                SL[pl.ds((part * D + d) * SS, NC), :] = s[32 * h:32 * h + 32, 128 * part:128 * part + 128]

    def g_p1(p0, n):
        for q in range(n):
            p1_pair(p0 + q)
            yield

    SCU = cfg.get("SCU", 4)

    def g_scan(q0, n):
        for it in range(q0, q0 + n):
            st = []
            for q in range(SCU):
                d0 = (it * SCU + q) * 8
                st.append([d0, mu[0, pl.ds(d0, 8), :], mu[1, pl.ds(d0, 8), :],
                           mu[2, pl.ds(d0, 8), :], mu[3, pl.ds(d0, 8), :], None, None])
            for c in range(NC):
                for q in range(SCU):
                    d0, mr, mi, sr, si, pr, pi = st[q]
                    if c >= 1:
                        lr = SL[pl.ds(d0 * SS + c - 1, 8, stride=SS), :]
                        li = SL[pl.ds((D + d0) * SS + c - 1, 8, stride=SS), :]
                        if c == 1:
                            sr, si = lr, li
                        else:
                            sr, si = mr * sr - mi * si + lr, mr * si + mi * sr + li
                    if c % 2 == 1:
                        S2[pl.ds(d0 * US + c // 2, 8, stride=US), :] = pltpu.pack_elementwise([pr, sr], packed_dtype=bf16)
                        S2[pl.ds((D + d0) * US + c // 2, 8, stride=US), :] = pltpu.pack_elementwise([pi, si], packed_dtype=bf16)
                    st[q] = [d0, mr, mi, sr, si, sr, si]
                if c % 8 == 7:
                    yield
    NSC = D // 8 // SCU

    def p2_pout(p, Vb):
        lr = [S2[pl.ds((p + 256 * h) * US, 16), :] for h in range(2)]
        li = [S2[pl.ds((D + p + 256 * h) * US, 16), :] for h in range(2)]
        lhs = pltpu.bitcast(jnp.concatenate([jnp.concatenate(lr, axis=0), jnp.concatenate(li, axis=0)], axis=1), bf16)
        return lax.dot_general(lhs, Vb, (((1,), (1,)), ((), ())), preferred_element_type=f32)

    def p2_tz(o):
        yi = jnp.where(lane32 < 64, o[0:32], o[32:64])
        krow = yi[0:1, :]
        tz = pltpu.roll(jnp.broadcast_to(krow, (64, 128)), 0, axis=1, stride=1, stride_axis=0)
        tzb = pltpu.bitcast(tz.astype(bf16), u32)
        T2 = pltpu.bitcast(jnp.concatenate([tzb & msk[0], tzb & msk[1]], axis=0), bf16)
        yi = jnp.concatenate([jnp.where(row8 == 0, 0.0, yi[0:8]), yi[8:32]], axis=0)
        return T2, yi

    def p2_intra(p, T2, yi):
        u = pltpu.bitcast(U[pl.ds(p * US, 16), :], bf16)
        y = jnp.dot(u, T2, preferred_element_type=f32) + yi
        Y[pl.ds(p * US, 16), :] = pltpu.bitcast(y.astype(bf16), u32)

    def g_p2(p0, n):
        V, O, T = {}, {}, {}
        nt = n + sum(G2)

        def it():
            for t in range(nt):
                q = t - sum(G2)
                if 0 <= q < n:
                    p2_intra(p0 + q, *T.pop(q))
                q = t - G2[0] - G2[1]
                if 0 <= q < n:
                    T[q] = p2_tz(O.pop(q))
                q = t - G2[0]
                if 0 <= q < n:
                    O[q] = p2_pout(p0 + q, V.pop(q))
                q = t
                if 0 <= q < n:
                    V[q] = vgen(p0 + q, False)
                yield
        return it(), nt

    def mlp_steps(b, first, last):
        r0 = b * MB
        xn = pltpu.bitcast(xnb[pl.ds(r0 // 2, MB // 2), :], bf16)
        acc = None
        for f in range(NF):
            if first:
                cp_w1(f).wait()
                w1c = w1s[:, f * FC:(f + 1) * FC]
                w1p[:, f * FC:(f + 1) * FC] = pltpu.bitcast(w1c, u32)
            else:
                w1c = pltpu.bitcast(w1p[:, f * FC:(f + 1) * FC], bf16)
            h = jnp.dot(xn, w1c, preferred_element_type=f32) + b1[:, f * FC:(f + 1) * FC]
            yield
            t = jnp.tanh((h * h * c12 + c1) * h)
            g = (h * t + h).astype(bf16)
            if first:
                cp_w2(f).wait()
                w2c = w2s[f * FC:(f + 1) * FC, :]
                w2p[pl.ds(f * FC // 2, FC // 2), :] = pltpu.bitcast(w2c, u32)
            else:
                w2c = pltpu.bitcast(w2p[pl.ds(f * FC // 2, FC // 2), :], bf16)
            a = jnp.dot(g, w2c, preferred_element_type=f32)
            acc = a if acc is None else acc + a
            yield
        res = acc * 0.5 + (xs[pl.ds(r0, MB), :].astype(f32) + xn.astype(f32) * dsk + b2)
        if last:
            for kk_ in range(MB // 128):
                k = b * (MB // 128) + kk_
                ob[pl.ds(k * 128, 128), :] = (res[kk_ * 128:(kk_ + 1) * 128] + y_rows(k)).astype(bf16)
            cp_o(b).start()
        else:
            ACC[pl.ds(r0, MB), :] = res
        yield
    NM = 2 * NF + 1

    def y_rows(k):
        ys = [[None] * 4, [None] * 4]
        for g in range(2):
            t = Y[pl.ds(g * 128 * US + k, 128, stride=US), :].T
            for cc in range(2):
                yv = pltpu.unpack_elementwise(t, index=cc, packed_dtype=bf16, unpacked_dtype=f32)
                ys[cc][g] = yv[0:64]
                ys[cc][g + 2] = yv[64:128]
        return jnp.concatenate([jnp.concatenate(ys[0], axis=1), jnp.concatenate(ys[1], axis=1)], axis=0)

    def g_final(blocks):
        for b in blocks:
            for k in range(b * (MB // 128), (b + 1) * (MB // 128)):
                ob[pl.ds(k * 128, 128), :] = (ACC[pl.ds(k * 128, 128), :] + y_rows(k)).astype(bf16)
                yield
            cp_o(b).start()

    def M(b):
        return mlp_steps(b, b == 0, b == NB - 1), NM

    plan = cfg.get("plan", "A")
    if plan == "A":
        interleave((g_ln([0]), 2))
        interleave(M(0), (g_ln([1]), 2))
        interleave(M(1), (g_ln(range(2, NB)), 2 * (NB - 2)))
        interleave(M(2), (g_param(), D // PR))
        interleave(M(3), (g_p1(0, NP), NP))
        interleave(M(4), (g_scan(0, NSC), NSC * 4))
        interleave(M(5), g_p2(0, NP // 2))
        interleave(M(6), g_p2(NP // 2, NP // 2))
        interleave(M(7), (g_final(range(NB - 1)), 2 * (NB - 1)))
    elif plan == "B":
        interleave((g_ln([0]), 2))
        interleave(M(0), (g_ln([1]), 2))
        interleave(M(1), chain((g_ln(range(2, NB)), 2 * (NB - 2)), (g_param(), D // PR)))
        interleave(M(2), (g_p1(0, NP), NP))
        interleave(M(3), (g_scan(0, NSC), NSC * 4))
        a, b_ = 86, 170
        interleave(M(4), g_p2(0, a))
        interleave(M(5), g_p2(a, b_ - a))
        interleave(M(6), g_p2(b_, NP - b_))
        interleave(M(7), (g_final(range(NB - 1)), 2 * (NB - 1)))

    for b in range(NB):
        cp_o(b).wait()


def build(**cfg):
    def fn(A_u, A_A_re, A_A_im, A_B_re, A_B_im, A_C_re, A_C_im, A_log_dt, A_Dskip, B_x, B_w1, B_b1, B_w2, B_b2):
        k = functools.partial(kernel, cfg=cfg)
        any_spec = pl.BlockSpec(memory_space=pl.ANY)
        out = pl.pallas_call(
            k,
            out_shape=jax.ShapeDtypeStruct((L, D), bf16),
            in_specs=[any_spec] * 13,
            out_specs=any_spec,
            scratch_shapes=[
                pltpu.VMEM((L, D), bf16),
                pltpu.VMEM((6, D, N), bf16),
                pltpu.VMEM((D,), bf16),
                pltpu.VMEM((D,), bf16),
                pltpu.VMEM((D,), bf16),
                pltpu.VMEM((F,), bf16),
                pltpu.VMEM((D, F), bf16),
                pltpu.VMEM((F, D), bf16),
                pltpu.VMEM((D // 2, F), u32),
                pltpu.VMEM((F // 2, D), u32),
                pltpu.VMEM((L // 2, D), u32),
                pltpu.VMEM((256 * US + 8, 128), u32),
                pltpu.VMEM((32 * TS + 8, 128), f32),
                pltpu.VMEM((2, D, 128), f32),
                pltpu.VMEM((4, D, 128), f32),
                pltpu.VMEM((2 * D * SS + 8, 128), f32),
                pltpu.VMEM((2 * D * US + 8, 128), u32),
                pltpu.VMEM((256 * US + 8, 128), u32),
                pltpu.VMEM((2, 32, 128), u32),
                pltpu.VMEM((L, D), f32),
                pltpu.VMEM((L, D), bf16),
                pltpu.SemaphoreType.DMA((NB,)),
                pltpu.SemaphoreType.DMA((NF,)),
                pltpu.SemaphoreType.DMA((NF,)),
                pltpu.SemaphoreType.DMA((6,)),
                pltpu.SemaphoreType.DMA((4,)),
                pltpu.SemaphoreType.DMA((NB,)),
            ],
            compiler_params=pltpu.CompilerParams(vmem_limit_bytes=110 * 2**20),
            name="k3",
        )(A_u.reshape(L, D), A_A_re, A_A_im, A_B_re, A_B_im, A_C_re, A_C_im, A_log_dt, A_Dskip,
          B_w1, B_b1, B_w2, B_b2)
        return out.reshape(1, L, D)
    return fn


_impl = build(**dict(plan='A'))


@jax.jit
def pallas_parallel_sum__ssm_conv_s4__mixer_channel_mlp__prompt_kernel(
    A_u: jax.Array,
    A_A_re: jax.Array,
    A_A_im: jax.Array,
    A_B_re: jax.Array,
    A_B_im: jax.Array,
    A_C_re: jax.Array,
    A_C_im: jax.Array,
    A_log_dt: jax.Array,
    A_Dskip: jax.Array,
    B_x: jax.Array,
    B_w1: jax.Array,
    B_b1: jax.Array,
    B_w2: jax.Array,
    B_b2: jax.Array,
):
    return _impl(A_u, A_A_re, A_A_im, A_B_re, A_B_im, A_C_re, A_C_im, A_log_dt, A_Dskip,
                 B_x, B_w1, B_b1, B_w2, B_b2)
```

```python
import functools
import jax
import jax.numpy as jnp
from jax import lax
import jax.experimental.pallas as pl
import jax.experimental.pallas.tpu as pltpu

f32, bf16, u32, i32 = jnp.float32, jnp.bfloat16, jnp.uint32, jnp.int32

L, D, N, F = 2048, 512, 128, 1792
Q, NC = 64, 32
TS = 513
US = 17
SS = 33
MB = 256
NB = L // MB
FC = 256
NF = F // FC
NP = 256


def cmul(ar, ai, br, bi):
    return ar * br - ai * bi, ar * bi + ai * br


def csq(ar, ai):
    return ar * ar - ai * ai, (ar * ai) * 2.0


def sincos(x):
    k = jnp.round(x * 0.6366197723675814)
    r = ((x - k * 1.5703125) - k * 4.837512969970703125e-4) - k * 7.54978995489188e-8
    z = r * r
    s = r + r * z * (-1.6666654611e-1 + z * (8.3321608736e-3 + z * -1.9515295891e-4))
    c = 1.0 + z * (-0.5 + z * (4.166664568298827e-2 + z * (-1.388731625493765e-3 + z * 2.443315711809948e-5)))
    q = k.astype(i32)
    swap = (q & 1) == 1
    sn = jnp.where(swap, c, s)
    cs = jnp.where(swap, s, c)
    sn = jnp.where((q & 2) == 2, -sn, sn)
    cs = jnp.where(((q + 1) & 2) == 2, -cs, cs)
    return sn, cs


def interleave(*gens):
    gens = [(g[0], g[1], g[2] if len(g) > 2 else (0.0, 1.0)) for g in gens if g[1] > 0]
    done = [0] * len(gens)
    total = sum(g[1] for g in gens)
    for _ in range(total):
        best = min((i for i in range(len(gens)) if done[i] < gens[i][1]),
                   key=lambda i: gens[i][2][0] + (gens[i][2][1] - gens[i][2][0]) * (done[i] + 0.5) / gens[i][1])
        next(gens[best][0])
        done[best] += 1
    for g, n, _r in gens:
        for _ in g:
            raise RuntimeError("generator not exhausted")


def chain(*gens):
    def it():
        for g, n in gens:
            for _ in range(n):
                next(g)
                yield
            for _ in g:
                raise RuntimeError("generator not exhausted")
    return it(), sum(n for _, n in gens)


def kernel(x_hbm, are_hbm, aim_hbm, bre_hbm, bim_hbm, cre_hbm, cim_hbm, ldt_hbm, dsk_hbm,
           w1_hbm, b1_hbm, w2_hbm, b2_hbm, o_hbm,
           xs, prm, v_ldt, v_dsk, v_b2, b1s, dtc_ref, mark_buf, w1s, w2s, w1p, w2p, xnb, U, tab, l8, mu, SL, S2, Y, msk, ACC, ob,
           sems, *, cfg):
    G2 = cfg.get("G2", (1, 4, 6))
    alag = cfg.get("alag", 0)

    p_hbm = [are_hbm, aim_hbm, bre_hbm, bim_hbm, cre_hbm, cim_hbm]
    vec = [v_ldt, v_dsk, v_b2, b1s]
    v_hbm = [ldt_hbm, dsk_hbm, b2_hbm, b1_hbm]

    def item(name, dz=None):
        k, i = name[0], int(name[1:] or 0)

        def off(step):
            return i * step if dz is None else pl.multiple_of(i * step + dz * step, step)

        if k == "x":
            return [(x_hbm.at[pl.ds(i * MB, MB)], xs[i])]
        if k == "a":
            return [(w1_hbm.at[:, pl.ds(i * FC, FC)], w1s[i])]
        if k == "b":
            return [(w2_hbm.at[pl.ds(i * FC, FC)], w2s[i])]
        if k == "p":
            return [(p_hbm[j], prm[j]) for j in range(6)]
        if k == "v":
            return [(v_hbm[j], vec[j]) for j in range(4)]
        if k == "o":
            return [(ob.at[pl.ds(i * MB, MB)], o_hbm.at[pl.ds(i * MB, MB)])]

    DMA_PLANS = {
        "g": {"t0": ["x0+v+a0"], "x0+v+a0": ["b0", "a1", "b1"],
              "b0": ["a2"], "a1": ["b2"], "b1": ["a3"], "a2": ["b3+x1"], "b2": ["a4"], "a3": ["b4"],
              "b3+x1": ["a5"], "a4": ["b5"], "b4": ["a6"], "a5": ["b6"],
              "b6": ["x2", "x3", "x4"], "x2": ["x5"], "x3": ["x6"], "x4": ["x7"], "x5": ["p"]},
        "h": {"t0": ["x0+v+a0", "b0+a1"], "x0+v+a0": ["b1", "a2"],
              "b0+a1": ["b2"], "b1": ["a3"], "a2": ["b3+x1"], "b2": ["a4"], "a3": ["b4"],
              "b3+x1": ["a5"], "a4": ["b5"], "b4": ["a6"], "a5": ["b6"],
              "a6": ["x2"], "b6": ["x3", "x4"], "x2": ["x5"], "x3": ["x6"], "x4": ["x7"], "x5": ["p"]},
    }
    DMA_PLANS["i"] = {"t0": ["x0+v+a0+b0"], "x0+v+a0+b0": ["a1+b1", "a2+b2", "a3+b3+x1", "a4+b4", "a5+b5", "a6+b6"],
              "a3+b3+x1": ["x2", "x3"], "a5+b5": ["x4", "x5"], "x2": ["x6"], "x3": ["x7"], "x4": ["p"]}
    DMA_PLANS["z"] = {"t0": ["x0+v+a0+b0+a1+b1+a2+b2+a3+b3+a4+b4+a5+b5+a6+b6+x1"],
                      "x0+v+a0+b0+a1+b1+a2+b2+a3+b3+a4+b4+a5+b5+a6+b6+x1": ["x2", "x3", "x4", "x5", "x6", "x7", "p"]}
    DMA_PLANS["y"] = {"t0": ["x0+v+a0"]+[c + str(f) for f in range(7) for c in "ab"][1:] + ["x1", "x2", "x3", "x4", "x5", "x6", "x7", "p"]}
    DMA_PLANS["w"] = {"t0": ["x0+v+a0", "x1", "b0"] + [c + str(f) for f in range(1, 7) for c in "ab"] + ["x2", "x3", "x4", "x5", "x6", "x7", "p"]}
    DMA_PLANS["w2"] = {"t0": ["x0+v+a0+x1+b0"], "x0+v+a0+x1+b0": [c + str(f) for f in range(1, 7) for c in "ab"] + ["x2", "x3", "x4", "x5", "x6", "x7", "p"]}
    DMA_PLANS["w3"] = {"t0": ["x0+v+a0"], "x0+v+a0": ["x1", "b0", "a1"], "x1": ["b1"], "b0": ["a2"], "a1": ["b2"],
                       "b1": ["a3"], "a2": ["b3"], "b2": ["x2"], "a3": ["a4"], "b3": ["b4"], "a4": ["x3", "a5"], "b4": ["b5", "x4"],
                       "a5": ["a6", "x5"], "b5": ["b6", "x6"], "a6": ["x7"], "b6": ["p"]}
    DMA_PLANS["y2"] = {"t0": ["x0+v+a0", "b0", "a1", "b1", "x1", "a2", "b2", "a3", "b3", "a4", "b4", "a5", "b5", "a6", "b6"],
                       "b4": ["x2"], "b5": ["x3", "x4"], "a6": ["x5"], "b6": ["x6", "x7"], "x3": ["p"]}
    DMA_PLANS["y3"] = {"t0": ["x0+v+a0", "b0", "a1", "b1", "x1", "a2", "b2", "a3", "b3", "a4", "b4", "a5", "b5", "a6", "b6"],
                       "b2": ["x2"], "b3": ["x3"], "b4": ["x4"], "a5": ["x5"], "b5": ["x6"], "a6": ["x7"], "b6": ["p"]}
    DMA_PLANS["w4"] = {"t0": ["x0+v", "a0", "x1", "b0"] + [c + str(f) for f in range(1, 7) for c in "ab"] + ["x2", "x3", "x4", "x5", "x6", "x7", "p"]}
    DMA_PLANS["w5"] = {"t0": ["x0+v", "a0", "x1", "b0"] + [c + str(f) for f in range(1, 4) for c in "ab"] + ["x2", "a4", "b4", "x3", "x4", "a5", "b5", "x5", "x6", "a6", "b6", "x7", "p"]}
    DMA_PLANS["w6"] = {"t0": ["x0+v+a0", "x1", "b0", "a1", "b1", "a2", "b2", "x2", "a3", "b3", "x3", "a4", "b4", "x4", "x5", "a5", "b5", "x6", "a6", "b6", "x7", "p"]}
    DMA_PLANS["w7"] = {"t0": ["x0+v+a0", "x1", "b0", "a1", "b1", "x2", "a2", "b2", "x3", "a3", "b3", "x4", "x5", "a4", "b4", "x6", "x7", "a5", "b5", "p", "a6", "b6"]}
    DMA_PLANS["s1"] = {"t0": ["x0+v+a0", "x1+b0", "a1+b1", "a2+b2+x2", "a3+b3+x3+x4", "a4+b4+x5+x6", "a5+b5+x7+p", "a6+b6"]}
    DMA_PLANS["s2"] = {"t0": ["x0+v+a0+b0", "x1+a1+b1", "a2+b2+x2+x3", "a3+b3+a4+b4+x4+x5", "a5+b5+a6+b6+x6+x7+p"]}
    DMA_PLANS["s3"] = {"t0": ["x0+v+x1+a0+b0", "a1+b1+a2+b2", "a3+b3+a4+b4+x2+x3+x4", "a5+b5+a6+b6+x5+x6+x7+p"]}
    DMA_PLANS["s4"] = {"t0": ["x0+v+a0", "x1+b0", "a1+b1", "a2+b2", "a3+b3+x2", "a4+b4+x3+x4", "a5+b5+x5+x6", "a6+b6+x7+p"]}
    DMA_PLANS["s5"] = {"t0": ["x0+v+a0", "x1+b0", "a1+b1", "a2+b2+x2", "a3+b3+x3", "a4+b4+x4+x5", "a5+b5+x6+x7", "a6+b6+p"]}
    DMA_PLANS["s6"] = {"t0": ["x0+v+a0", "x1", "b0", "a1+b1", "a2+b2+x2", "a3+b3+x3+x4", "a4+b4+x5+x6", "a5+b5+x7", "a6+b6+p"]}
    dma_plan = cfg.get("dma", "g")
    dma_plan = DMA_PLANS[dma_plan] if isinstance(dma_plan, str) else dma_plan
    groups = sorted({g for v in dma_plan.values() for g in v}) + ["o%d" % b for b in range(NB)]
    sem_of = {g: i for i, g in enumerate(groups)}
    member = {it: g for g in groups for it in g.split("+")}
    state = {}

    hist = []

    marks = []
    arrived = {}

    def sem_ref(g, pin):
        idx = sem_of[g]
        if pin is not None:
            t = pltpu.bitcast(pin, i32)[0, 0]
            idx = idx + (((t * t) & 2) >> 1)
        return sems.at[idx]

    def copies(g, sem):
        return [pltpu.make_async_copy(src, dst, sem) for it in g.split("+") for src, dst in item(it)]

    def start(g):
        assert g not in state, g
        state[g] = 1
        for c in copies(g, sems.at[sem_of[g]]):
            c.start()

    def trigger(key):
        for g in dma_plan.get(key, []):
            start(g)

    def need(it):
        g = member[it]
        assert g in state, it
        if state[g] == 1:
            state[g] = 2
            lag = cfg.get("pin", 0)
            if lag and len(hist) >= lag and g[0] != "o":
                t = pltpu.bitcast(hist[-lag], i32)[0, 0]
                dz = ((t * t) & 2) >> 1
                n = len(marks)
                marks.append(pltpu.make_async_copy(are_hbm.at[pl.ds(pl.multiple_of(dz * 16, 16), 16)],
                                                   mark_buf.at[pl.ds(16 * n, 16)], sems.at[len(groups)]))
                marks[-1].start()
            for c in copies(g, sems.at[sem_of[g]]):
                c.wait()
            trigger(g)
        return arrived.get(g)

    def at(start, z, m):
        return start if z is None else pl.multiple_of(start + z, m)

    trigger("t0")

    z = jnp.uint32(0)
    kk = lax.broadcasted_iota(i32, (32, 128), 0) * 2
    ln = lax.broadcasted_iota(i32, (32, 128), 1)
    lo = jnp.uint32(0x0000FFFF)
    hi = jnp.uint32(0xFFFF0000)
    for h in range(2):
        inh = (ln >= 64 * h) & (ln < 64 * h + 64)
        li = ln - 64 * h
        msk[h] = jnp.where(inh & (li >= kk), lo, z) | jnp.where(inh & (li >= kk + 1), hi, z)
    lane = lax.broadcasted_iota(i32, (16, 128), 1)
    laneA = jnp.where(lane < 64, jnp.uint32(0xFFFFFFFF), z)
    lane32 = lax.broadcasted_iota(i32, (32, 128), 1)
    row8 = lax.broadcasted_iota(i32, (8, 128), 0)
    c1 = 0.7978845608028654
    c12 = 0.7978845608028654 * 0.044715

    need("v")
    dsk = v_dsk[...].astype(f32).reshape(1, D)
    b2 = v_b2[...].astype(f32).reshape(1, D)
    b1 = b1s[...].astype(f32).reshape(1, F)

    sbits = pltpu.bitcast(b2, i32)[0, 0]
    TRUE = ((sbits * sbits) & 2) == 0
    pending = []
    tick = [0]

    def anchor(*vals):
        for v in vals:
            pending.append((tick[0], v if v.dtype == u32 else pltpu.bitcast(v, u32)))

    def take(w, th, tw, maxn=None):
        tick[0] += 1
        n = sum(1 for t_, _ in pending if tick[0] - t_ > alag)
        if maxn is not None:
            n = min(maxn, n)
        if n == 0:
            return w
        R, C = w.shape
        ntile = (R // th) * (C // tw)
        vals = [pending.pop(0)[1] for _ in range(n)]
        slots = {}
        for i, v in enumerate(vals):
            t = (i * ntile) // n
            slots.setdefault(t, []).append(v)
        rows = []
        for kt in range(R // th):
            cols = []
            for nt in range(C // tw):
                t = kt * (C // tw) + nt
                blk = w[th * kt:th * kt + th, tw * nt:tw * nt + tw]
                vs = slots.get(t, [])
                if vs:
                    assert tw == 128
                    while len(vs) > th // 8:
                        a = vs.pop()
                        vs[-1] = vs[-1] | a
                    parts = []
                    nv = th // 8
                    for j in range(nv):
                        piece = blk[8 * j:8 * j + 8]
                        k = j - (nv - len(vs))
                        if k >= 0:
                            piece = jnp.where(TRUE, piece, vs[k])
                        parts.append(piece)
                    blk = jnp.concatenate(parts, axis=0)
                cols.append(blk)
            rows.append(jnp.concatenate(cols, axis=1) if len(cols) > 1 else cols[0])
        return jnp.concatenate(rows, axis=0) if len(rows) > 1 else rows[0]

    def ln_rows(k, z):
        r0 = k * 128
        x = xs[r0 // MB][pl.ds(r0 % MB, 128), :].astype(f32)
        m = jnp.mean(x, axis=-1, keepdims=True)
        xc = x - m
        v = jnp.mean(xc * xc, axis=-1, keepdims=True)
        xn = xc * lax.rsqrt(v + 1e-5)
        xnb[pl.ds(r0 // 2, 64), :] = pltpu.bitcast(xn.astype(bf16), u32)
        if k < 2:
            hist.append(xn[120:128, 384:512])
        pk = pltpu.pack_elementwise([xn[0:64], xn[64:128]], packed_dtype=bf16)
        for g in range(2):
            t = jnp.concatenate([pk[:, 128 * g:128 * g + 128], pk[:, 128 * (g + 2):128 * (g + 2) + 128]], axis=0)
            U[pl.ds(g * 128 * US + k, 128, stride=US), :] = t.T

    def g_ln(blocks):
        for b in blocks:
            z = need("x%d" % b)
            for k in (2 * b, 2 * b + 1):
                ln_rows(k, z)
                yield

    def param_rows(r0, R, anc):
        sl = pl.ds(r0, R)
        sz = pl.ds(at(r0, pz[0], R), R)
        dtb = dtc_ref[sl, :]
        ar = dtb * prm[0][sl, :].astype(f32)
        ai = dtb * prm[1][sl, :].astype(f32)
        dbr = dtb * prm[2][sl, :].astype(f32)
        dbi = dtb * prm[3][sl, :].astype(f32)
        wr, wi = cmul(prm[4][sl, :].astype(f32), prm[5][sl, :].astype(f32), dbr, dbi)
        wi = -wi
        e = jnp.exp(ar)
        sn, cs = sincos(ai)
        l1r, l1i = e * cs, e * sn
        l2r, l2i = csq(l1r, l1i)
        l4r, l4i = csq(l2r, l2i)
        l8r, l8i = csq(l4r, l4i)
        l3r, l3i = cmul(l2r, l2i, l1r, l1i)
        l5r, l5i = cmul(l4r, l4i, l1r, l1i)
        l6r, l6i = cmul(l4r, l4i, l2r, l2i)
        l7r, l7i = cmul(l4r, l4i, l3r, l3i)
        pw = [(jnp.ones_like(ar), jnp.zeros_like(ar)), (l1r, l1i), (l2r, l2i), (l3r, l3i),
              (l4r, l4i), (l5r, l5i), (l6r, l6i), (l7r, l7i), (l8r, l8i)]
        for s in range(8):
            tab[pl.ds((2 * 8 + s) * TS + r0, R), :] = pw[s][0]
            tab[pl.ds((3 * 8 + s) * TS + r0, R), :] = pw[s][1]
            pr, pi = pw[8 - s]
            t0_, t1_ = wr * pr + wi * pi, wi * pr - wr * pi
            tab[pl.ds((0 * 8 + s) * TS + r0, R), :] = t0_
            tab[pl.ds((1 * 8 + s) * TS + r0, R), :] = t1_
            if anc == 2:
                for j in range(R // 8):
                    anchor(t0_[8 * j:8 * j + 8] + t1_[8 * j:8 * j + 8])
        l8[0, sl, :] = l8r
        l8[1, sl, :] = l8i
        mr, mi = csq(l8r, l8i)
        mr, mi = csq(mr, mi)
        mr, mi = csq(mr, mi)
        mu[0, sl, :] = mr
        mu[1, sl, :] = -mi
        mu[2, sl, :] = wr
        mu[3, sl, :] = wi
        if anc:
            for j in range(R // 8):
                anchor(mr[8 * j:8 * j + 8])

    PR = 16

    dtc_box = []
    pz = [None]

    def get_dtc():
        if not dtc_box:
            dt_row = jnp.exp(v_ldt[...].astype(f32).reshape(1, D)).astype(bf16).astype(f32)
            dtc_ref[...] = jnp.broadcast_to(dt_row, (128, D)).T
            dtc_box.append(1)

    def g_param(rows, anc, wait):
        pz[0] = need("p")
        for r0 in rows:
            param_rows(r0, PR, anc)
            yield

    def PARAM(p0, n, anc=False, wait=False):
        rows = [h * 256 + p0 + PR * i for i in range(n // PR) for h in range(2)]
        return g_param(rows, anc, wait), len(rows)

    def bc(ref, part, d):
        return jnp.broadcast_to(ref[part, pl.ds(d, 1), :], (8, 128))

    def vgen(p, conj):
        t0 = 0 if conj else 2
        r_l, i_l = [], []
        for h in range(2):
            d = p + 256 * h
            tr = tab[pl.ds(t0 * 8 * TS + d, 8, stride=TS), :]
            ti = tab[pl.ds((t0 + 1) * 8 * TS + d, 8, stride=TS), :]
            sr, si = bc(l8, 0, d), bc(l8, 1, d)
            rs, is_ = [tr], [ti]
            for v in range(7):
                if conj:
                    tr, ti = tr * sr + ti * si, ti * sr - tr * si
                else:
                    tr, ti = tr * sr - ti * si, tr * si + ti * sr
                rs.append(tr)
                is_.append(ti)
            if conj:
                rs, is_ = rs[::-1], is_[::-1]
            r_l += rs
            i_l += is_
        return jnp.concatenate([jnp.concatenate(r_l, axis=0), jnp.concatenate(i_l, axis=0)], axis=1).astype(bf16)

    def p1_pair(p):
        Wb = vgen(p, True)
        if pending and cfg.get("take_p1", 0):
            Wb = pltpu.bitcast(take(pltpu.bitcast(Wb, u32), 64, 128, cfg["take_p1"]), bf16)
        u = U[pl.ds(p * US, 16), :]
        ua = u & laneA
        ub = u ^ ua
        lhs = pltpu.bitcast(jnp.concatenate([ua, ub], axis=0), bf16)
        s = jnp.dot(lhs, Wb, preferred_element_type=f32)
        for h in range(2):
            d = p + 256 * h
            for part in range(2):
                SL[pl.ds((part * D + d) * SS, NC), :] = s[32 * h:32 * h + 32, 128 * part:128 * part + 128]

    def g_p1(p0, n):
        for q in range(n):
            p1_pair(p0 + q)
            yield

    SCU = cfg.get("SCU", 4)

    def g_scan(groups, sgran, anc):
        for g0 in range(0, len(groups), SCU):
            st = []
            for d0 in groups[g0:g0 + SCU]:
                st.append([d0, mu[0, pl.ds(d0, 8), :], mu[1, pl.ds(d0, 8), :],
                           mu[2, pl.ds(d0, 8), :], mu[3, pl.ds(d0, 8), :], None, None])
            for c in range(NC):
                for q in range(len(st)):
                    d0, mr, mi, sr, si, pr, pi = st[q]
                    if c >= 1:
                        lr = SL[pl.ds(d0 * SS + c - 1, 8, stride=SS), :]
                        li = SL[pl.ds((D + d0) * SS + c - 1, 8, stride=SS), :]
                        if c == 1:
                            sr, si = lr, li
                        else:
                            sr, si = mr * sr - mi * si + lr, mr * si + mi * sr + li
                    if c % 2 == 1:
                        S2[pl.ds(d0 * US + c // 2, 8, stride=US), :] = pltpu.pack_elementwise([pr, sr], packed_dtype=bf16)
                        S2[pl.ds((D + d0) * US + c // 2, 8, stride=US), :] = pltpu.pack_elementwise([pi, si], packed_dtype=bf16)
                    st[q] = [d0, mr, mi, sr, si, sr, si]
                if c % sgran == sgran - 1:
                    if anc:
                        anchor(*[x[3] for x in st])
                    yield

    def SCAN(p0, n, sgran=8, anc=False):
        groups = [h * 256 + p0 + 8 * i for i in range(n // 8) for h in range(2)]
        return g_scan(groups, sgran, anc), (len(groups) // SCU) * (NC // sgran)

    def p2_pout(p, Vb):
        lr = [S2[pl.ds((p + 256 * h) * US, 16), :] for h in range(2)]
        li = [S2[pl.ds((D + p + 256 * h) * US, 16), :] for h in range(2)]
        lhs = pltpu.bitcast(jnp.concatenate([jnp.concatenate(lr, axis=0), jnp.concatenate(li, axis=0)], axis=1), bf16)
        return lax.dot_general(lhs, Vb, (((1,), (1,)), ((), ())), preferred_element_type=f32)

    def p2_tz(o):
        yi = jnp.where(lane32 < 64, o[0:32], o[32:64])
        krow = yi[0:1, :]
        tz = pltpu.roll(jnp.broadcast_to(krow, (64, 128)), 0, axis=1, stride=1, stride_axis=0)
        tzb = pltpu.bitcast(tz.astype(bf16), u32)
        T2 = pltpu.bitcast(jnp.concatenate([tzb & msk[0], tzb & msk[1]], axis=0), bf16)
        yi = jnp.concatenate([jnp.where(row8 == 0, 0.0, yi[0:8]), yi[8:32]], axis=0)
        return T2, yi

    def p2_intra(p, T2, yi):
        u = pltpu.bitcast(U[pl.ds(p * US, 16), :], bf16)
        y = jnp.dot(u, T2, preferred_element_type=f32) + yi
        Y[pl.ds(p * SS, NC), :] = y

    def g_p2(p0, n):
        V, O, T = {}, {}, {}
        nt = n + sum(G2)

        def it():
            for t in range(nt):
                q = t - sum(G2)
                if 0 <= q < n:
                    p2_intra(p0 + q, *T.pop(q))
                q = t - G2[0] - G2[1]
                if 0 <= q < n:
                    T[q] = p2_tz(O.pop(q))
                q = t - G2[0]
                if 0 <= q < n:
                    O[q] = p2_pout(p0 + q, V.pop(q))
                q = t
                if 0 <= q < n:
                    V[q] = vgen(p0 + q, False)
                    if pending and cfg.get("take_p2", 0):
                        V[q] = pltpu.bitcast(take(pltpu.bitcast(V[q], u32), 64, 128, cfg["take_p2"]), bf16)
                yield
        return it(), nt

    def mlp_steps(b, first, last):
        conv = first and first_blocks[b] == 2
        r0 = b * MB
        xn = pltpu.bitcast(xnb[pl.ds(r0 // 2, MB // 2), :], bf16)
        acc = None
        for f in range(NF):
            if first:
                z = need("a%d" % f)
                w1c = w1s[f][...]
                if conv:
                    w1p[:, f * FC:(f + 1) * FC] = pltpu.bitcast(w1c, u32)
            else:
                w1c = pltpu.bitcast(take(w1p[:, f * FC:(f + 1) * FC], 64, 128), bf16)
            h = jnp.dot(xn, w1c, preferred_element_type=f32) + b1[:, f * FC:(f + 1) * FC]
            hist.append(h[MB - 8:MB, FC - 128:FC])
            yield
            t = jnp.tanh((h * h * c12 + c1) * h)
            g = (h * t + h).astype(bf16)
            if first:
                z = need("b%d" % f)
                w2c = w2s[f][...]
                if conv:
                    w2p[pl.ds(f * FC // 2, FC // 2), :] = pltpu.bitcast(w2c, u32)
            else:
                w2c = pltpu.bitcast(take(w2p[pl.ds(f * FC // 2, FC // 2), :], 64, 128), bf16)
            a = jnp.dot(g, w2c, preferred_element_type=f32)
            acc = a if acc is None else acc + a
            hist.append(a[MB - 8:MB, D - 128:D])
            yield
        res = acc * 0.5 + (xs[b][...].astype(f32) + xn.astype(f32) * dsk + b2)
        if last:
            for kk_ in range(MB // 128):
                k = b * (MB // 128) + kk_
                ob[pl.ds(k * 128, 128), :] = (res[kk_ * 128:(kk_ + 1) * 128] + y_rows(k)).astype(bf16)
            start("o%d" % b)
        else:
            ACC[pl.ds(r0, MB), :] = res
        yield
    NM = 2 * NF + 1

    def y_rows(k):
        ys = [[None] * 4, [None] * 4]
        for g in range(2):
            for cc in range(2):
                yv = Y[pl.ds(g * 128 * SS + 2 * k + cc, 128, stride=SS), :].T
                ys[cc][g] = yv[0:64]
                ys[cc][g + 2] = yv[64:128]
        return jnp.concatenate([jnp.concatenate(ys[0], axis=1), jnp.concatenate(ys[1], axis=1)], axis=0)

    def g_final(blocks, anc):
        for b in blocks:
            for k in range(b * (MB // 128), (b + 1) * (MB // 128)):
                r_ = (ACC[pl.ds(k * 128, 128), :] + y_rows(k)).astype(bf16)
                ob[pl.ds(k * 128, 128), :] = r_
                if anc:
                    r32 = pltpu.bitcast(r_, u32)
                    anchor(r32[0:8, 0:128], r32[0:8, 128:256], r32[32:40, 256:384], r32[32:40, 384:512])
                if k % (MB // 128) == (MB // 128) - 1:
                    start("o%d" % b)
                yield

    direct = set(cfg.get("direct", [NB - 1]))
    first_blocks = cfg.get("first_blocks", {0: 2})

    def M(b):
        return mlp_steps(b, b in first_blocks, b in direct), NM

    def LN(blocks):
        blocks = list(blocks)
        return g_ln(blocks), 2 * len(blocks)

    def P1(p0, n):
        return g_p1(p0, n), n

    def FIN(blocks, anc=False):
        blocks = list(blocks)
        return g_final(blocks, anc), 2 * len(blocks)

    def DTC():
        def it():
            get_dtc()
            yield
        return it(), 1

    nstage = [0]

    def stage(*gens):
        nstage[0] += 1
        t = sbits + nstage[0]
        if nstage[0] in cfg.get("nobr", ()):
            del pending[:]
            interleave(*gens)
            del pending[:]
            return

        @pl.when(((t * t) & 2) == 0)
        def _():
            del pending[:]
            if cfg.get("scope"):
                with jax.named_scope("stage%d" % nstage[0]):
                    interleave(*gens)
            else:
                interleave(*gens)
            del pending[:]

    plan = cfg.get("plan", "A")
    sg = cfg.get("sgran", 2)
    pa = cfg.get("panc", 1)
    if plan == "A":
        interleave(LN([0]))
        stage(M(0), LN([1]) + (cfg.get('ln1', (0.75, 0.9)),))
        stage(M(1), LN(range(2, NB)) + (cfg.get('lnr', (0.0, 1.0)),))
        stage(M(2), chain(DTC(), PARAM(0, 256, wait=True)))
        stage(M(3), P1(0, 256))
        stage(M(4), SCAN(0, 256))
        stage(M(5), g_p2(0, 128))
        stage(M(6), g_p2(128, 128))
        stage(M(7), FIN(range(NB - 1), cfg.get("fanc", 0)))
    elif plan == "D":
        interleave(LN([0]))
        stage(M(0), LN([1]) + (cfg.get('ln1', (0.75, 0.9)),))
        stage(M(1), LN(range(2, NB)) + (cfg.get('lnr', (0.0, 1.0)),))
        stage(M(2), chain(DTC(), PARAM(0, 128, anc=pa, wait=True)))
        stage(M(3), P1(0, 128), PARAM(128, 128, anc=pa))
        stage(M(4), P1(128, 128), SCAN(0, 128, sg, True))
        stage(M(5), g_p2(0, 128), SCAN(128, 128, sg, True))
        stage(M(6), g_p2(128, 128))
        stage(M(7), FIN(range(NB - 1), cfg.get("fanc", 0)))
    elif plan == "G":
        interleave(LN([0]))
        stage(M(0), M(1) + ((0.03, 1.0),), LN([1]) + ((0.0, 0.03),))
        stage(M(2), LN(range(2, NB)) + ((0.0, 0.6),), chain(DTC(), PARAM(0, 128, anc=pa, wait=True)) + ((0.3, 1.0),))
        stage(M(3), P1(0, 128), PARAM(128, 128, anc=pa))
        stage(M(4), P1(128, 128), SCAN(0, 128, sg, True))
        stage(M(5), g_p2(0, 128), SCAN(128, 128, sg, True))
        stage(M(6), g_p2(128, 128))
        stage(M(7), FIN(range(NB - 1), cfg.get("fanc", 0)))
    elif plan == "F":
        interleave(LN([0]))
        stage(M(0), M(1) + ((0.03, 1.0),), LN([1]) + ((0.0, 0.03),), LN(range(2, NB)) + (cfg.get('lnr', (0.55, 1.0)),), DTC() + ((0.1, 0.12),))
        stage(M(2), PARAM(0, 128, anc=pa, wait=True) + (cfg.get("prange", (0.0, 1.0)),))
        stage(M(3), P1(0, 128), PARAM(128, 128, anc=pa))
        stage(M(4), P1(128, 128), SCAN(0, 128, sg, True))
        stage(M(5), g_p2(0, 128), SCAN(128, 128, sg, True))
        stage(M(6), g_p2(128, 128))
        stage(M(7), FIN(range(NB - 1), cfg.get("fanc", 0)))
    elif plan == "E":
        interleave(LN([0]))
        stage(M(0), LN([1]) + (cfg.get('ln1', (0.75, 0.9)),))
        stage(M(1), LN(range(2, NB)) + (cfg.get('lnr', (0.0, 1.0)),))
        stage(M(2), chain(DTC(), PARAM(0, 128, anc=pa, wait=True)))
        stage(M(3), P1(0, 128), PARAM(128, 128, anc=pa))
        stage(M(4), P1(128, 128), SCAN(0, 128, sg, True))
        stage(M(5), g_p2(0, 128), SCAN(128, 128, sg, True))
        stage(M(6), g_p2(128, 128))
        stage(M(7), FIN(range(NB - 1), cfg.get("fanc", 0)))

    for n in range(len(marks)):
        pltpu.make_async_copy(are_hbm.at[pl.ds(0, 16)], mark_buf.at[pl.ds(16 * n, 16)], sems.at[len(groups)]).wait()
    for b in range(NB):
        need("o%d" % b)
    assert all(state.get(g) == 2 for g in groups), state


def build(**cfg):
    def fn(A_u, A_A_re, A_A_im, A_B_re, A_B_im, A_C_re, A_C_im, A_log_dt, A_Dskip, B_x, B_w1, B_b1, B_w2, B_b2):
        k = functools.partial(kernel, cfg=cfg)
        any_spec = pl.BlockSpec(memory_space=pl.ANY)
        out = pl.pallas_call(
            k,
            out_shape=jax.ShapeDtypeStruct((L, D), bf16),
            grid=(1,),
            in_specs=[any_spec] * 13,
            out_specs=any_spec,
            scratch_shapes=[
                [pltpu.VMEM((MB, D), bf16)] * NB,
                [pltpu.VMEM((D, N), bf16)] * 6,
                pltpu.VMEM((D,), bf16),
                pltpu.VMEM((D,), bf16),
                pltpu.VMEM((D,), bf16),
                pltpu.VMEM((F,), bf16),
                pltpu.VMEM((D, 128), f32),
                pltpu.VMEM((16 * 32, 128), bf16),
                [pltpu.VMEM((D, FC), bf16)] * NF,
                [pltpu.VMEM((FC, D), bf16)] * NF,
                pltpu.VMEM((D // 2, F), u32),
                pltpu.VMEM((F // 2, D), u32),
                pltpu.VMEM((L // 2, D), u32),
                pltpu.VMEM((256 * US + 8, 128), u32),
                pltpu.VMEM((32 * TS + 8, 128), f32),
                pltpu.VMEM((2, D, 128), f32),
                pltpu.VMEM((4, D, 128), f32),
                pltpu.VMEM((2 * D * SS + 8, 128), f32),
                pltpu.VMEM((2 * D * US + 8, 128), u32),
                pltpu.VMEM((256 * SS + 8, 128), f32),
                pltpu.VMEM((2, 32, 128), u32),
                pltpu.VMEM((L, D), f32),
                pltpu.VMEM((L, D), bf16),
                pltpu.SemaphoreType.DMA((40,)),
            ],
            compiler_params=pltpu.CompilerParams(vmem_limit_bytes=110 * 2**20, **({'flags': cfg['flags']} if cfg.get('flags') else {})),
            name="k4",
        )(A_u.reshape(L, D), A_A_re, A_A_im, A_B_re, A_B_im, A_C_re, A_C_im, A_log_dt, A_Dskip,
          B_w1, B_b1, B_w2, B_b2)
        return out.reshape(1, L, D)
    return fn


_impl = build(**dict(flags={'XLA_TPU_RESCHEDULE_DMA_DONES': True}, plan='F', nobr=(1,2,3,4,5,6,7), fanc=1, sgran=4, G2=(1,8,8), SCU=8,panc=1, take_p1=2, take_p2=2, pin=2, dma='s5', lnr=(0.3,0.95)))


@jax.jit
def pallas_parallel_sum__ssm_conv_s4__mixer_channel_mlp__prompt_kernel(
    A_u: jax.Array,
    A_A_re: jax.Array,
    A_A_im: jax.Array,
    A_B_re: jax.Array,
    A_B_im: jax.Array,
    A_C_re: jax.Array,
    A_C_im: jax.Array,
    A_log_dt: jax.Array,
    A_Dskip: jax.Array,
    B_x: jax.Array,
    B_w1: jax.Array,
    B_b1: jax.Array,
    B_w2: jax.Array,
    B_b2: jax.Array,
):
    return _impl(A_u, A_A_re, A_A_im, A_B_re, A_B_im, A_C_re, A_C_im, A_log_dt, A_Dskip,
                 B_x, B_w1, B_b1, B_w2, B_b2)
```

```python
import functools
import jax
import jax.numpy as jnp
from jax import lax
import jax.experimental.pallas as pl
import jax.experimental.pallas.tpu as pltpu

f32, bf16, u32, i32 = jnp.float32, jnp.bfloat16, jnp.uint32, jnp.int32

L, D, N, F = 2048, 512, 128, 1792
Q, NC = 64, 32
TS = 513
US = 17
SS = 33
MB = 256
NB = L // MB
FC = 256
NF = F // FC
NP = 256


def cmul(ar, ai, br, bi):
    return ar * br - ai * bi, ar * bi + ai * br


def csq(ar, ai):
    return ar * ar - ai * ai, (ar * ai) * 2.0


def sincos(x):
    k = jnp.round(x * 0.6366197723675814)
    r = ((x - k * 1.5703125) - k * 4.837512969970703125e-4) - k * 7.54978995489188e-8
    z = r * r
    s = r + r * z * (-1.6666654611e-1 + z * (8.3321608736e-3 + z * -1.9515295891e-4))
    c = 1.0 + z * (-0.5 + z * (4.166664568298827e-2 + z * (-1.388731625493765e-3 + z * 2.443315711809948e-5)))
    q = k.astype(i32)
    swap = (q & 1) == 1
    sn = jnp.where(swap, c, s)
    cs = jnp.where(swap, s, c)
    sn = jnp.where((q & 2) == 2, -sn, sn)
    cs = jnp.where(((q + 1) & 2) == 2, -cs, cs)
    return sn, cs


def interleave(*gens):
    gens = [(g[0], g[1], g[2] if len(g) > 2 else (0.0, 1.0)) for g in gens if g[1] > 0]
    done = [0] * len(gens)
    total = sum(g[1] for g in gens)
    for _ in range(total):
        best = min((i for i in range(len(gens)) if done[i] < gens[i][1]),
                   key=lambda i: gens[i][2][0] + (gens[i][2][1] - gens[i][2][0]) * (done[i] + 0.5) / gens[i][1])
        next(gens[best][0])
        done[best] += 1
    for g, n, _r in gens:
        for _ in g:
            raise RuntimeError("generator not exhausted")


def chain(*gens):
    def it():
        for g, n in gens:
            for _ in range(n):
                next(g)
                yield
            for _ in g:
                raise RuntimeError("generator not exhausted")
    return it(), sum(n for _, n in gens)


def kernel(x_hbm, are_hbm, aim_hbm, bre_hbm, bim_hbm, cre_hbm, cim_hbm, ldt_hbm, dsk_hbm,
           w1_hbm, b1_hbm, w2_hbm, b2_hbm, o_hbm,
           xs, prm, v_ldt, v_dsk, v_b2, b1s, dtc_ref, mark_buf, w1s, w2s, w1p, w2p, xnb, U, tab, l8, mu, SL, S2, Y, msk, ACC, ob,
           sems, *, cfg):
    G2 = cfg.get("G2", (1, 4, 6))
    alag = cfg.get("alag", 0)

    p_hbm = [are_hbm, aim_hbm, bre_hbm, bim_hbm, cre_hbm, cim_hbm]
    vec = [v_ldt, v_dsk, v_b2, b1s]
    v_hbm = [ldt_hbm, dsk_hbm, b2_hbm, b1_hbm]

    def item(name, dz=None):
        k, i = name[0], int(name[1:] or 0)

        def off(step):
            return i * step if dz is None else pl.multiple_of(i * step + dz * step, step)

        if k == "x":
            return [(x_hbm.at[pl.ds(i * MB, MB)], xs[i])]
        if k == "a":
            return [(w1_hbm.at[:, pl.ds(i * FC, FC)], w1s[i])]
        if k == "b":
            return [(w2_hbm.at[pl.ds(i * FC, FC)], w2s[i])]
        if k == "p":
            return [(p_hbm[j], prm[j]) for j in range(6)]
        if k == "v":
            return [(v_hbm[j], vec[j]) for j in range(4)]
        if k == "o":
            return [(ob.at[pl.ds(i * MB, MB)], o_hbm.at[pl.ds(i * MB, MB)])]

    dma_plan = {"t0": ["x0+v+a0", "x1+b0", "a1+b1", "a2+b2+x2", "a3+b3+x3",
                       "a4+b4+x4+x5", "a5+b5+x6+x7", "a6+b6+p"]}
    groups = sorted({g for v in dma_plan.values() for g in v}) + ["o%d" % b for b in range(NB)]
    sem_of = {g: i for i, g in enumerate(groups)}
    member = {it: g for g in groups for it in g.split("+")}
    state = {}

    hist = []

    marks = []
    arrived = {}

    def copies(g, sem):
        return [pltpu.make_async_copy(src, dst, sem) for it in g.split("+") for src, dst in item(it)]

    def start(g):
        assert g not in state, g
        state[g] = 1
        for c in copies(g, sems.at[sem_of[g]]):
            c.start()

    def trigger(key):
        for g in dma_plan.get(key, []):
            start(g)

    def need(it):
        g = member[it]
        assert g in state, it
        if state[g] == 1:
            state[g] = 2
            lag = cfg.get("pin", 0)
            if lag and len(hist) >= lag and g[0] != "o":
                t = pltpu.bitcast(hist[-lag], i32)[0, 0]
                dz = ((t * t) & 2) >> 1
                n = len(marks)
                marks.append(pltpu.make_async_copy(are_hbm.at[pl.ds(pl.multiple_of(dz * 16, 16), 16)],
                                                   mark_buf.at[pl.ds(16 * n, 16)], sems.at[len(groups)]))
                marks[-1].start()
            for c in copies(g, sems.at[sem_of[g]]):
                c.wait()
            trigger(g)
        return arrived.get(g)

    def at(start, z, m):
        return start if z is None else pl.multiple_of(start + z, m)

    trigger("t0")

    z = jnp.uint32(0)
    kk = lax.broadcasted_iota(i32, (32, 128), 0) * 2
    ln = lax.broadcasted_iota(i32, (32, 128), 1)
    lo = jnp.uint32(0x0000FFFF)
    hi = jnp.uint32(0xFFFF0000)
    for h in range(2):
        inh = (ln >= 64 * h) & (ln < 64 * h + 64)
        li = ln - 64 * h
        msk[h] = jnp.where(inh & (li >= kk), lo, z) | jnp.where(inh & (li >= kk + 1), hi, z)
    lane = lax.broadcasted_iota(i32, (16, 128), 1)
    laneA = jnp.where(lane < 64, jnp.uint32(0xFFFFFFFF), z)
    lane32 = lax.broadcasted_iota(i32, (32, 128), 1)
    row8 = lax.broadcasted_iota(i32, (8, 128), 0)
    c1 = 0.7978845608028654
    c12 = 0.7978845608028654 * 0.044715

    need("v")
    dsk = v_dsk[...].astype(f32).reshape(1, D)
    b2 = v_b2[...].astype(f32).reshape(1, D)
    b1 = b1s[...].astype(f32).reshape(1, F)

    sbits = pltpu.bitcast(b2, i32)[0, 0]
    TRUE = ((sbits * sbits) & 2) == 0
    pending = []
    tick = [0]

    def anchor(*vals):
        for v in vals:
            pending.append((tick[0], v if v.dtype == u32 else pltpu.bitcast(v, u32)))

    def take(w, th, tw, maxn=None):
        tick[0] += 1
        n = sum(1 for t_, _ in pending if tick[0] - t_ > alag)
        if maxn is not None:
            n = min(maxn, n)
        if n == 0:
            return w
        R, C = w.shape
        ntile = (R // th) * (C // tw)
        vals = [pending.pop(0)[1] for _ in range(n)]
        slots = {}
        for i, v in enumerate(vals):
            t = (i * ntile) // n
            slots.setdefault(t, []).append(v)
        rows = []
        for kt in range(R // th):
            cols = []
            for nt in range(C // tw):
                t = kt * (C // tw) + nt
                blk = w[th * kt:th * kt + th, tw * nt:tw * nt + tw]
                vs = slots.get(t, [])
                if vs:
                    assert tw == 128
                    while len(vs) > th // 8:
                        a = vs.pop()
                        vs[-1] = vs[-1] | a
                    parts = []
                    nv = th // 8
                    for j in range(nv):
                        piece = blk[8 * j:8 * j + 8]
                        k = j - (nv - len(vs))
                        if k >= 0:
                            piece = jnp.where(TRUE, piece, vs[k])
                        parts.append(piece)
                    blk = jnp.concatenate(parts, axis=0)
                cols.append(blk)
            rows.append(jnp.concatenate(cols, axis=1) if len(cols) > 1 else cols[0])
        return jnp.concatenate(rows, axis=0) if len(rows) > 1 else rows[0]

    def ln_rows(k, z):
        r0 = k * 128
        x = xs[r0 // MB][pl.ds(r0 % MB, 128), :].astype(f32)
        m = jnp.mean(x, axis=-1, keepdims=True)
        xc = x - m
        v = jnp.mean(xc * xc, axis=-1, keepdims=True)
        xn = xc * lax.rsqrt(v + 1e-5)
        xnb[pl.ds(r0 // 2, 64), :] = pltpu.bitcast(xn.astype(bf16), u32)
        if k < 2:
            hist.append(xn[120:128, 384:512])
        pk = pltpu.pack_elementwise([xn[0:64], xn[64:128]], packed_dtype=bf16)
        for g in range(2):
            t = jnp.concatenate([pk[:, 128 * g:128 * g + 128], pk[:, 128 * (g + 2):128 * (g + 2) + 128]], axis=0)
            U[pl.ds(g * 128 * US + k, 128, stride=US), :] = t.T

    def g_ln(blocks):
        for b in blocks:
            z = need("x%d" % b)
            for k in (2 * b, 2 * b + 1):
                ln_rows(k, z)
                yield

    def param_rows(r0, R, anc):
        sl = pl.ds(r0, R)
        sz = pl.ds(at(r0, pz[0], R), R)
        dtb = dtc_ref[sl, :]
        ar = dtb * prm[0][sl, :].astype(f32)
        ai = dtb * prm[1][sl, :].astype(f32)
        dbr = dtb * prm[2][sl, :].astype(f32)
        dbi = dtb * prm[3][sl, :].astype(f32)
        wr, wi = cmul(prm[4][sl, :].astype(f32), prm[5][sl, :].astype(f32), dbr, dbi)
        wi = -wi
        e = jnp.exp(ar)
        sn, cs = sincos(ai)
        l1r, l1i = e * cs, e * sn
        l2r, l2i = csq(l1r, l1i)
        l4r, l4i = csq(l2r, l2i)
        l8r, l8i = csq(l4r, l4i)
        l3r, l3i = cmul(l2r, l2i, l1r, l1i)
        l5r, l5i = cmul(l4r, l4i, l1r, l1i)
        l6r, l6i = cmul(l4r, l4i, l2r, l2i)
        l7r, l7i = cmul(l4r, l4i, l3r, l3i)
        pw = [(jnp.ones_like(ar), jnp.zeros_like(ar)), (l1r, l1i), (l2r, l2i), (l3r, l3i),
              (l4r, l4i), (l5r, l5i), (l6r, l6i), (l7r, l7i), (l8r, l8i)]
        for s in range(8):
            tab[pl.ds((2 * 8 + s) * TS + r0, R), :] = pw[s][0]
            tab[pl.ds((3 * 8 + s) * TS + r0, R), :] = pw[s][1]
            pr, pi = pw[8 - s]
            t0_, t1_ = wr * pr + wi * pi, wi * pr - wr * pi
            tab[pl.ds((0 * 8 + s) * TS + r0, R), :] = t0_
            tab[pl.ds((1 * 8 + s) * TS + r0, R), :] = t1_
            if anc == 2:
                for j in range(R // 8):
                    anchor(t0_[8 * j:8 * j + 8] + t1_[8 * j:8 * j + 8])
        l8[0, sl, :] = l8r
        l8[1, sl, :] = l8i
        mr, mi = csq(l8r, l8i)
        mr, mi = csq(mr, mi)
        mr, mi = csq(mr, mi)
        mu[0, sl, :] = mr
        mu[1, sl, :] = -mi
        mu[2, sl, :] = wr
        mu[3, sl, :] = wi
        if anc:
            for j in range(R // 8):
                anchor(mr[8 * j:8 * j + 8])

    PR = 16

    dtc_box = []
    pz = [None]

    def get_dtc():
        if not dtc_box:
            dt_row = jnp.exp(v_ldt[...].astype(f32).reshape(1, D)).astype(bf16).astype(f32)
            dtc_ref[...] = jnp.broadcast_to(dt_row, (128, D)).T
            dtc_box.append(1)

    def g_param(rows, anc, wait):
        pz[0] = need("p")
        for r0 in rows:
            param_rows(r0, PR, anc)
            yield

    def PARAM(p0, n, anc=False, wait=False):
        rows = [h * 256 + p0 + PR * i for i in range(n // PR) for h in range(2)]
        return g_param(rows, anc, wait), len(rows)

    def bc(ref, part, d):
        return jnp.broadcast_to(ref[part, pl.ds(d, 1), :], (8, 128))

    def vgen(p, conj):
        t0 = 0 if conj else 2
        r_l, i_l = [], []
        for h in range(2):
            d = p + 256 * h
            tr = tab[pl.ds(t0 * 8 * TS + d, 8, stride=TS), :]
            ti = tab[pl.ds((t0 + 1) * 8 * TS + d, 8, stride=TS), :]
            sr, si = bc(l8, 0, d), bc(l8, 1, d)
            rs, is_ = [tr], [ti]
            for v in range(7):
                if conj:
                    tr, ti = tr * sr + ti * si, ti * sr - tr * si
                else:
                    tr, ti = tr * sr - ti * si, tr * si + ti * sr
                rs.append(tr)
                is_.append(ti)
            if conj:
                rs, is_ = rs[::-1], is_[::-1]
            r_l += rs
            i_l += is_
        return jnp.concatenate([jnp.concatenate(r_l, axis=0), jnp.concatenate(i_l, axis=0)], axis=1).astype(bf16)

    def p1_pair(p):
        Wb = vgen(p, True)
        if pending and cfg.get("take_p1", 0):
            Wb = pltpu.bitcast(take(pltpu.bitcast(Wb, u32), 64, 128, cfg["take_p1"]), bf16)
        u = U[pl.ds(p * US, 16), :]
        ua = u & laneA
        ub = u ^ ua
        lhs = pltpu.bitcast(jnp.concatenate([ua, ub], axis=0), bf16)
        s = jnp.dot(lhs, Wb, preferred_element_type=f32)
        for h in range(2):
            d = p + 256 * h
            for part in range(2):
                SL[pl.ds((part * D + d) * SS, NC), :] = s[32 * h:32 * h + 32, 128 * part:128 * part + 128]

    def g_p1(p0, n):
        for q in range(n):
            p1_pair(p0 + q)
            yield

    SCU = cfg.get("SCU", 4)

    def g_scan(groups, sgran, anc):
        for g0 in range(0, len(groups), SCU):
            st = []
            for d0 in groups[g0:g0 + SCU]:
                st.append([d0, mu[0, pl.ds(d0, 8), :], mu[1, pl.ds(d0, 8), :],
                           mu[2, pl.ds(d0, 8), :], mu[3, pl.ds(d0, 8), :], None, None])
            for c in range(NC):
                for q in range(len(st)):
                    d0, mr, mi, sr, si, pr, pi = st[q]
                    if c >= 1:
                        lr = SL[pl.ds(d0 * SS + c - 1, 8, stride=SS), :]
                        li = SL[pl.ds((D + d0) * SS + c - 1, 8, stride=SS), :]
                        if c == 1:
                            sr, si = lr, li
                        else:
                            sr, si = mr * sr - mi * si + lr, mr * si + mi * sr + li
                    if c % 2 == 1:
                        S2[pl.ds(d0 * US + c // 2, 8, stride=US), :] = pltpu.pack_elementwise([pr, sr], packed_dtype=bf16)
                        S2[pl.ds((D + d0) * US + c // 2, 8, stride=US), :] = pltpu.pack_elementwise([pi, si], packed_dtype=bf16)
                    st[q] = [d0, mr, mi, sr, si, sr, si]
                if c % sgran == sgran - 1:
                    if anc:
                        anchor(*[x[3] for x in st])
                    yield

    def SCAN(p0, n, sgran=8, anc=False):
        groups = [h * 256 + p0 + 8 * i for i in range(n // 8) for h in range(2)]
        return g_scan(groups, sgran, anc), (len(groups) // SCU) * (NC // sgran)

    def p2_pout(p, Vb):
        lr = [S2[pl.ds((p + 256 * h) * US, 16), :] for h in range(2)]
        li = [S2[pl.ds((D + p + 256 * h) * US, 16), :] for h in range(2)]
        lhs = pltpu.bitcast(jnp.concatenate([jnp.concatenate(lr, axis=0), jnp.concatenate(li, axis=0)], axis=1), bf16)
        return lax.dot_general(lhs, Vb, (((1,), (1,)), ((), ())), preferred_element_type=f32)

    def p2_tz(o):
        yi = jnp.where(lane32 < 64, o[0:32], o[32:64])
        krow = yi[0:1, :]
        tz = pltpu.roll(jnp.broadcast_to(krow, (64, 128)), 0, axis=1, stride=1, stride_axis=0)
        tzb = pltpu.bitcast(tz.astype(bf16), u32)
        T2 = pltpu.bitcast(jnp.concatenate([tzb & msk[0], tzb & msk[1]], axis=0), bf16)
        yi = jnp.concatenate([jnp.where(row8 == 0, 0.0, yi[0:8]), yi[8:32]], axis=0)
        return T2, yi

    def p2_intra(p, T2, yi):
        u = pltpu.bitcast(U[pl.ds(p * US, 16), :], bf16)
        y = jnp.dot(u, T2, preferred_element_type=f32) + yi
        Y[pl.ds(p * SS, NC), :] = y

    def g_p2(p0, n):
        V, O, T = {}, {}, {}
        nt = n + sum(G2)

        def it():
            for t in range(nt):
                q = t - sum(G2)
                if 0 <= q < n:
                    p2_intra(p0 + q, *T.pop(q))
                q = t - G2[0] - G2[1]
                if 0 <= q < n:
                    T[q] = p2_tz(O.pop(q))
                q = t - G2[0]
                if 0 <= q < n:
                    O[q] = p2_pout(p0 + q, V.pop(q))
                q = t
                if 0 <= q < n:
                    V[q] = vgen(p0 + q, False)
                    if pending and cfg.get("take_p2", 0):
                        V[q] = pltpu.bitcast(take(pltpu.bitcast(V[q], u32), 64, 128, cfg["take_p2"]), bf16)
                yield
        return it(), nt

    def mlp_steps(b, first, last):
        conv = first and first_blocks[b] == 2
        r0 = b * MB
        xn = pltpu.bitcast(xnb[pl.ds(r0 // 2, MB // 2), :], bf16)
        acc = None
        for f in range(NF):
            if first:
                z = need("a%d" % f)
                w1c = w1s[f][...]
                if conv:
                    w1p[:, f * FC:(f + 1) * FC] = pltpu.bitcast(w1c, u32)
            else:
                w1c = pltpu.bitcast(take(w1p[:, f * FC:(f + 1) * FC], 64, 128), bf16)
            h = jnp.dot(xn, w1c, preferred_element_type=f32) + b1[:, f * FC:(f + 1) * FC]
            hist.append(h[MB - 8:MB, FC - 128:FC])
            yield
            t = jnp.tanh((h * h * c12 + c1) * h)
            g = (h * t + h).astype(bf16)
            if first:
                z = need("b%d" % f)
                w2c = w2s[f][...]
                if conv:
                    w2p[pl.ds(f * FC // 2, FC // 2), :] = pltpu.bitcast(w2c, u32)
            else:
                w2c = pltpu.bitcast(take(w2p[pl.ds(f * FC // 2, FC // 2), :], 64, 128), bf16)
            a = jnp.dot(g, w2c, preferred_element_type=f32)
            acc = a if acc is None else acc + a
            hist.append(a[MB - 8:MB, D - 128:D])
            yield
        res = acc * 0.5 + (xs[b][...].astype(f32) + xn.astype(f32) * dsk + b2)
        if last:
            for kk_ in range(MB // 128):
                k = b * (MB // 128) + kk_
                ob[pl.ds(k * 128, 128), :] = (res[kk_ * 128:(kk_ + 1) * 128] + y_rows(k)).astype(bf16)
            start("o%d" % b)
        else:
            ACC[pl.ds(r0, MB), :] = res
        yield
    NM = 2 * NF + 1

    def y_rows(k):
        ys = [[None] * 4, [None] * 4]
        for g in range(2):
            for cc in range(2):
                yv = Y[pl.ds(g * 128 * SS + 2 * k + cc, 128, stride=SS), :].T
                ys[cc][g] = yv[0:64]
                ys[cc][g + 2] = yv[64:128]
        return jnp.concatenate([jnp.concatenate(ys[0], axis=1), jnp.concatenate(ys[1], axis=1)], axis=0)

    def g_final(blocks, anc):
        for b in blocks:
            for k in range(b * (MB // 128), (b + 1) * (MB // 128)):
                r_ = (ACC[pl.ds(k * 128, 128), :] + y_rows(k)).astype(bf16)
                ob[pl.ds(k * 128, 128), :] = r_
                if anc:
                    r32 = pltpu.bitcast(r_, u32)
                    anchor(r32[0:8, 0:128], r32[0:8, 128:256], r32[32:40, 256:384], r32[32:40, 384:512])
                if k % (MB // 128) == (MB // 128) - 1:
                    start("o%d" % b)
                yield

    direct = set(cfg.get("direct", [NB - 1]))
    first_blocks = cfg.get("first_blocks", {0: 2})

    def M(b):
        return mlp_steps(b, b in first_blocks, b in direct), NM

    def LN(blocks):
        blocks = list(blocks)
        return g_ln(blocks), 2 * len(blocks)

    def P1(p0, n):
        return g_p1(p0, n), n

    def FIN(blocks, anc=False):
        blocks = list(blocks)
        return g_final(blocks, anc), 2 * len(blocks)

    def DTC():
        def it():
            get_dtc()
            yield
        return it(), 1

    nstage = [0]

    def stage(*gens):
        nstage[0] += 1
        t = sbits + nstage[0]
        if nstage[0] in cfg.get("nobr", ()):
            del pending[:]
            interleave(*gens)
            del pending[:]
            return

        @pl.when(((t * t) & 2) == 0)
        def _():
            del pending[:]
            if cfg.get("scope"):
                with jax.named_scope("stage%d" % nstage[0]):
                    interleave(*gens)
            else:
                interleave(*gens)
            del pending[:]

    plan = cfg.get("plan", "A")
    sg = cfg.get("sgran", 2)
    pa = cfg.get("panc", 1)
    if plan == "F":
        interleave(LN([0]))
        stage(M(0), M(1) + ((0.03, 1.0),), LN([1]) + ((0.0, 0.03),), LN(range(2, NB)) + (cfg.get('lnr', (0.55, 1.0)),), DTC() + ((0.1, 0.12),))
        stage(M(2), PARAM(0, 128, anc=pa, wait=True) + (cfg.get("prange", (0.0, 1.0)),))
        stage(M(3), P1(0, 128), PARAM(128, 128, anc=pa))
        stage(M(4), P1(128, 128), SCAN(0, 128, sg, True))
        stage(M(5), g_p2(0, 128), SCAN(128, 128, sg, True))
        stage(M(6), g_p2(128, 128))
        stage(M(7), FIN(range(NB - 1), cfg.get("fanc", 0)))

    for n in range(len(marks)):
        pltpu.make_async_copy(are_hbm.at[pl.ds(0, 16)], mark_buf.at[pl.ds(16 * n, 16)], sems.at[len(groups)]).wait()
    for b in range(NB):
        need("o%d" % b)
    assert all(state.get(g) == 2 for g in groups), state


def build(**cfg):
    def fn(A_u, A_A_re, A_A_im, A_B_re, A_B_im, A_C_re, A_C_im, A_log_dt, A_Dskip, B_x, B_w1, B_b1, B_w2, B_b2):
        k = functools.partial(kernel, cfg=cfg)
        any_spec = pl.BlockSpec(memory_space=pl.ANY)
        out = pl.pallas_call(
            k,
            out_shape=jax.ShapeDtypeStruct((L, D), bf16),
            grid=(1,),
            in_specs=[any_spec] * 13,
            out_specs=any_spec,
            scratch_shapes=[
                [pltpu.VMEM((MB, D), bf16)] * NB,
                [pltpu.VMEM((D, N), bf16)] * 6,
                pltpu.VMEM((D,), bf16),
                pltpu.VMEM((D,), bf16),
                pltpu.VMEM((D,), bf16),
                pltpu.VMEM((F,), bf16),
                pltpu.VMEM((D, 128), f32),
                pltpu.VMEM((16 * 32, 128), bf16),
                [pltpu.VMEM((D, FC), bf16)] * NF,
                [pltpu.VMEM((FC, D), bf16)] * NF,
                pltpu.VMEM((D // 2, F), u32),
                pltpu.VMEM((F // 2, D), u32),
                pltpu.VMEM((L // 2, D), u32),
                pltpu.VMEM((256 * US + 8, 128), u32),
                pltpu.VMEM((32 * TS + 8, 128), f32),
                pltpu.VMEM((2, D, 128), f32),
                pltpu.VMEM((4, D, 128), f32),
                pltpu.VMEM((2 * D * SS + 8, 128), f32),
                pltpu.VMEM((2 * D * US + 8, 128), u32),
                pltpu.VMEM((256 * SS + 8, 128), f32),
                pltpu.VMEM((2, 32, 128), u32),
                pltpu.VMEM((L, D), f32),
                pltpu.VMEM((L, D), bf16),
                pltpu.SemaphoreType.DMA((40,)),
            ],
            compiler_params=pltpu.CompilerParams(vmem_limit_bytes=110 * 2**20, **({'flags': cfg['flags']} if cfg.get('flags') else {})),
            name="ssm_mixer_k4",
        )(A_u.reshape(L, D), A_A_re, A_A_im, A_B_re, A_B_im, A_C_re, A_C_im, A_log_dt, A_Dskip,
          B_w1, B_b1, B_w2, B_b2)
        return out.reshape(1, L, D)
    return fn


_impl = build(**dict(flags={'XLA_TPU_RESCHEDULE_DMA_DONES': True}, plan='F', nobr=(1,2,3,4,5,6,7), fanc=1, sgran=4, G2=(1,8,8), SCU=8, panc=1, take_p1=2, take_p2=2, pin=2, lnr=(0.3,0.95)))


@jax.jit
def pallas_parallel_sum__ssm_conv_s4__mixer_channel_mlp__prompt_kernel(
    A_u: jax.Array,
    A_A_re: jax.Array,
    A_A_im: jax.Array,
    A_B_re: jax.Array,
    A_B_im: jax.Array,
    A_C_re: jax.Array,
    A_C_im: jax.Array,
    A_log_dt: jax.Array,
    A_Dskip: jax.Array,
    B_x: jax.Array,
    B_w1: jax.Array,
    B_b1: jax.Array,
    B_w2: jax.Array,
    B_b2: jax.Array,
):
    return _impl(A_u, A_A_re, A_A_im, A_B_re, A_B_im, A_C_re, A_C_im, A_log_dt, A_Dskip,
                 B_x, B_w1, B_b1, B_w2, B_b2)
```
